```python
import os as _os
_os.environ.setdefault("JAX_PLATFORMS", "cpu")
import jax
import jax.numpy as jnp

def _softmax(x, axis=-1):
    return jax.nn.softmax(x, axis=axis)
def _gelu(x):
    return jax.nn.gelu(x, approximate=True)
def _silu(x):
    return jax.nn.silu(x)
def _sigmoid(x):
    return jax.nn.sigmoid(x)
def _layernorm(x, axis=-1, eps=1e-5):
    m = jnp.mean(x, axis=axis, keepdims=True)
    v = jnp.var(x, axis=axis, keepdims=True)
    return (x - m) / jnp.sqrt(v + eps)
def _scatter_add(tgt, idx, src, axis=0):
    return tgt.at[idx].add(src)
def _segment_sum(src, seg, n):
    return jax.ops.segment_sum(src, seg, n)
class _Rng:
    def __init__(self, key):
        self._k = key
    def _next(self):
        self._k, sub = jax.random.split(self._k)
        return sub
    def normal(self, shape):
        return jax.random.normal(self._next(), shape, dtype=jnp.bfloat16)
    def randint(self, lo, hi, shape):
        return jax.random.randint(self._next(), shape, lo, hi, dtype=jnp.int32)
    def uniform(self, shape, lo=0.0, hi=1.0):
        return jax.random.uniform(self._next(), shape, jnp.bfloat16, lo, hi)
    def permutation(self, n):
        return jax.random.permutation(self._next(), n)


kernel_name = 'sequential_preLN__mha_block__dense_activation_mish__prompt'

def setup_inputs():
    _rng = _Rng(jax.random.key(int.from_bytes(__import__("os").urandom(4), "little")))
    _w = (lambda a: (lambda t: t.astype(jnp.bfloat16) if jnp.issubdtype(t.dtype, jnp.floating) else t)(jnp.asarray(a)))
    def _A_setup():
        B, S, D, H = 1, 2048, 576, 32
        return {
            "x": _w((lambda *s: _rng.normal(s) * 0.05)(B, S, D)),
            "wqkv": _w((lambda *s: _rng.normal(s) * 0.05)(D, 3 * D)),
            "wo": _w((lambda *s: _rng.normal(s) * 0.05)(D, D)),
        }
    _A_in = _A_setup()

    def _B_setup():
        B, S, D, F = 1, 2048, 576, 4608
        return {
            "x": _w((lambda *s: _rng.normal(s) * 0.05)(B, S, D)),
            "w1": _w((lambda *s: _rng.normal(s) * 1.6)(D, F) * (D ** -0.5)),
            "b1": _w((lambda *s: _rng.normal(s) * 0.05)(F)),
            "w2": _w((lambda *s: _rng.normal(s) * 0.05)(F, D) * (F ** -0.5)),
        }
    _B_in = _B_setup()

    return {
        "A_x": _A_in["x"],
        "A_wqkv": _A_in["wqkv"],
        "A_wo": _A_in["wo"],
        "B_x": _B_in["x"],
        "B_w1": _B_in["w1"],
        "B_b1": _B_in["b1"],
        "B_w2": _B_in["w2"],
    }

def reference(A_x, A_wqkv, A_wo, B_x, B_w1, B_b1, B_w2):
    def _A_ref(x, wqkv, wo):
        B, S, D = x.shape
        H = 32
        Dh = D // H
        qkv = (lambda x, *d: x.transpose(*d))((x @ wqkv).reshape(B, S, 3, H, Dh), 2, 0, 3, 1, 4)
        q, k, v = qkv[0], qkv[1], qkv[2]
        scores = jnp.einsum("bhqd,bhkd->bhqk", q, k) * (Dh ** -0.5)
        p = _softmax(scores, axis=-1)
        o = jnp.einsum("bhqk,bhkd->bhqd", p, v)
        return (lambda x, *d: x.transpose(*d))(o, 0, 2, 1, 3).reshape(B, S, D) @ wo

    def _B_ref(x, w1, b1, w2):
        h = jnp.einsum("bsd,df->bsf", x, w1) + b1
        sp = jnp.log1p(jnp.exp(-jnp.abs(h))) + jnp.where(h > 0, h, jnp.zeros_like(h))
        act = h * jnp.tanh(sp)
        return jnp.einsum("bsf,fd->bsd", act, w2)

    x = A_x
    h = x + _A_ref(_layernorm(x, axis=-1), A_wqkv, A_wo)
    h2 = h + _B_ref(_layernorm(h, axis=-1), B_w1, B_b1, B_w2)
    return h2
```

```python
import functools
import jax
import jax.numpy as jnp
import jax.experimental.pallas as pl
import jax.experimental.pallas.tpu as pltpu

S, D, H, DH, F = 2048, 576, 32, 18, 4608
EPS = 1e-5
f32, bf16 = jnp.float32, jnp.bfloat16
TN = (((0,), (0,)), ((), ()))
NT = (((1,), (1,)), ((), ()))

def _lnT(x):
    m = jnp.mean(x, axis=0, keepdims=True)
    xc = x - m
    v = jnp.mean(xc * xc, axis=0, keepdims=True)
    return xc * jax.lax.rsqrt(v + EPS)

def kernel(xT_hbm, wqkv_hbm, wo_hbm, w1_hbm, b1_hbm, w2T_hbm, oT_hbm,
           xT_ref, wqkv_ref, wo_ref, w1_ref, b1_ref, w2T_ref, oT_ref, sems, osem,
           wT_s, qT_s, k_s, vT_s, aT_s, s_buf, m_buf, *, tq, tr, tr3, phases):
    scale = DH ** -0.5
    nq = S // tq
    cps = [pltpu.make_async_copy(src, dst, sems.at[i]) for i, (src, dst) in enumerate(
        [(xT_hbm, xT_ref), (wqkv_hbm, wqkv_ref), (wo_hbm, wo_ref), (w1_hbm, w1_ref), (b1_hbm, b1_ref), (w2T_hbm, w2T_ref)])]
    for c in cps: c.start()
    cps[0].wait(); cps[1].wait()
    if 1 in phases:
      wT_s[...] = wqkv_ref[...].T
      for r in range(S // tr):
        cols = pl.ds(r * tr, tr)
        xnT = _lnT(xT_ref[:, cols].astype(f32)).astype(bf16)
        qkvT = jnp.dot(wT_s[...], xnT, preferred_element_type=f32)
        kk = qkvT[D:2 * D, :].T
        for h in range(H):
            qT_s[h, :, cols] = (qkvT[h * DH:(h + 1) * DH, :] * scale).astype(bf16)
            k_s[h, cols, :] = kk[:, h * DH:(h + 1) * DH].astype(bf16)
            vT_s[h, 0:DH, cols] = qkvT[2 * D + h * DH:2 * D + (h + 1) * DH, :].astype(bf16)
      ones_rows = jnp.concatenate([jnp.ones((1, S), bf16), jnp.zeros((5, S), bf16)], axis=0)
      for h in range(H):
        vT_s[h, DH:24, :] = ones_rows

    def stage_a(i, slot):
        h = i // nq
        cols = pl.ds(pl.multiple_of((i % nq) * tq, tq), tq)
        sT = jnp.dot(k_s[h], qT_s[h, :, cols], preferred_element_type=f32)
        s_buf[slot] = sT
        m_buf[slot] = jnp.max(sT, axis=0, keepdims=True)

    def stage_b(i, slot):
        h = i // nq
        cols = pl.ds(pl.multiple_of((i % nq) * tq, tq), tq)
        p = jnp.exp(s_buf[slot] - m_buf[slot]).astype(bf16)
        oT = jnp.dot(vT_s[h], p, preferred_element_type=f32)
        aT_s[h, :, cols] = oT[0:DH, :] / oT[DH:DH + 1, :]

    if 2 in phases:
      stage_a(0, 0)
      def body(j, c):
          i = 2 * j
          stage_a(i + 1, 1)
          stage_b(i, 0)
          stage_a(jnp.minimum(i + 2, H * nq - 1), 0)
          stage_b(i + 1, 1)
          return c
      jax.lax.fori_loop(0, H * nq // 2, body, 0)

    for c in cps[2:]: c.wait()
    ocs = []
    for r in range(S // tr3):
        cols = pl.ds(r * tr3, tr3)
        if 3 in phases:
          aT = aT_s[:, :, cols].reshape(D, tr3).astype(bf16)
          attnT = jax.lax.dot_general(wo_ref[...], aT, TN, preferred_element_type=f32)
          hT = xT_ref[:, cols].astype(f32) + attnT
          hn = _lnT(hT).T.astype(bf16)
          a = jnp.dot(hn, w1_ref[...], preferred_element_type=f32) + b1_ref[...].astype(f32)
          sp = jnp.log1p(jnp.exp(-jnp.abs(a))) + jnp.maximum(a, 0.0)
          act = (a * jnp.tanh(sp)).astype(bf16)
          yT = jax.lax.dot_general(w2T_ref[...], act, NT, preferred_element_type=f32)
          oT_ref[:, cols] = (hT + yT).astype(oT_ref.dtype)
        else:
          oT_ref[:, cols] = xT_ref[:, cols]
        oc = pltpu.make_async_copy(oT_ref.at[:, cols], oT_hbm.at[:, cols], osem.at[r])
        oc.start(); ocs.append(oc)
    for oc in ocs: oc.wait()


@jax.jit
def pallas_sequential_preLN__mha_block__dense_activation_mish__prompt_kernel(A_x, A_wqkv, A_wo, B_x, B_w1, B_b1, B_w2):
    tq, tr, tr3, phases = 1024, 512, 1024, (1, 2, 3)
    xT = jnp.transpose(A_x, (0, 2, 1)).reshape(D, S)
    b1 = B_b1.reshape(1, F)
    w2T = B_w2.T
    any_spec = pl.BlockSpec(memory_space=pl.ANY)
    outT = pl.pallas_call(
        functools.partial(kernel, tq=tq, tr=tr, tr3=tr3, phases=phases),
        out_shape=jax.ShapeDtypeStruct((D, S), A_x.dtype),
        in_specs=[any_spec] * 6,
        out_specs=any_spec,
        scratch_shapes=[
            pltpu.VMEM((D, S), bf16), pltpu.VMEM((D, 3 * D), bf16), pltpu.VMEM((D, D), bf16),
            pltpu.VMEM((D, F), bf16), pltpu.VMEM((1, F), bf16), pltpu.VMEM((D, F), bf16),
            pltpu.VMEM((D, S), bf16),
            pltpu.SemaphoreType.DMA((6,)), pltpu.SemaphoreType.DMA((S // tr3,)),
            pltpu.VMEM((3 * D, D), bf16),
            pltpu.VMEM((H, DH, S), bf16),
            pltpu.VMEM((H, S, DH), bf16),
            pltpu.VMEM((H, 24, S), bf16),
            pltpu.VMEM((H, DH, S), f32),
            pltpu.VMEM((2, S, tq), f32),
            pltpu.VMEM((2, 1, tq), f32),
        ],
        compiler_params=pltpu.CompilerParams(vmem_limit_bytes=120 * 1024 * 1024),
    )(xT, A_wqkv, A_wo, B_w1, b1, w2T)
    return jnp.transpose(outT.reshape(1, D, S), (0, 2, 1))
```
